```python
import jax
import jax.numpy as jnp

def _softmax(x, axis=-1):
    return jax.nn.softmax(x, axis=axis)
def _gelu(x):
    return jax.nn.gelu(x, approximate=True)
def _silu(x):
    return jax.nn.silu(x)
def _sigmoid(x):
    return jax.nn.sigmoid(x)
def _layernorm(x, axis=-1, eps=1e-5):
    m = jnp.mean(x, axis=axis, keepdims=True)
    v = jnp.var(x, axis=axis, keepdims=True)
    return (x - m) / jnp.sqrt(v + eps)
def _scatter_add(tgt, idx, src, axis=0):
    return tgt.at[idx].add(src)
def _segment_sum(src, seg, n):
    return jax.ops.segment_sum(src, seg, n)
class _Rng:
    def __init__(self, key):
        self._k = key
    def _next(self):
        self._k, sub = jax.random.split(self._k)
        return sub
    def normal(self, shape):
        return jax.random.normal(self._next(), shape, dtype=jnp.bfloat16)
    def randint(self, lo, hi, shape):
        return jax.random.randint(self._next(), shape, lo, hi, dtype=jnp.int32)
    def uniform(self, shape, lo=0.0, hi=1.0):
        return jax.random.uniform(self._next(), shape, jnp.bfloat16, lo, hi)
    def permutation(self, n):
        return jax.random.permutation(self._next(), n)


kernel_name = 'gated_mix__linear_attn_block__moe_arch_mod__prompt'

def setup_inputs():
    _rng = _Rng(jax.random.key(int.from_bytes(__import__("os").urandom(4), "little")))
    _w = (lambda a: (lambda t: t.astype(jnp.bfloat16) if jnp.issubdtype(t.dtype, jnp.floating) else t)(jnp.asarray(a)))
    def _A_setup():
        B, S, D = 1, 2048, 1024
        return {
            "x": _w((lambda *s: _rng.normal(s) * 0.05)(B, S, D)),
            "wqkv": _w((lambda *s: _rng.normal(s) * 0.05)(D, 3 * D)),
            "wo": _w((lambda *s: _rng.normal(s) * 0.05)(D, D)),
        }
    _A_in = _A_setup()

    def _B_setup():
        B, S, D, F, C = 1, 2048, 1024, 3584, 1
        return {
            "x": _w((lambda *s: _rng.normal(s) * 0.05)(B, S, D)),
            "w_r": _w((lambda *s: _rng.normal(s) * 0.05)(D)),
            "w_gate": _w((lambda *s: _rng.normal(s) * 0.05)(D, F)),
            "w_up": _w((lambda *s: _rng.normal(s) * 0.05)(D, F)),
            "w_down": _w((lambda *s: _rng.normal(s) * 0.05)(F, D)),
        }
    _B_in = _B_setup()

    return {
        "A_x": _A_in["x"],
        "A_wqkv": _A_in["wqkv"],
        "A_wo": _A_in["wo"],
        "B_x": _B_in["x"],
        "B_w_r": _B_in["w_r"],
        "B_w_gate": _B_in["w_gate"],
        "B_w_up": _B_in["w_up"],
        "B_w_down": _B_in["w_down"],
        "gate_w": _w((lambda *s: _rng.normal(s) * 0.05)(1024)),
    }

def reference(A_x, A_wqkv, A_wo, B_x, B_w_r, B_w_gate, B_w_up, B_w_down, gate_w):
    def _A_ref(x, wqkv, wo):
        B, S, D = x.shape
        H = 32; Dh = D // H
        qkv = (lambda x, *d: x.transpose(*d))((x @ wqkv).reshape(B, S, 3, H, Dh), 2, 0, 3, 1, 4)
        q, k, v = qkv[0], qkv[1], qkv[2]
        phi = lambda t: jnp.where(t > 0, t + 1, jnp.exp(t)) + 1e-6
        pq, pk = phi(q), phi(k)
        kv = jnp.einsum("bhsd,bhse->bhde", pk, v)
        z = jnp.einsum("bhsd->bhd", pk)
        num = jnp.einsum("bhqd,bhde->bhqe", pq, kv)
        den = jnp.einsum("bhqd,bhd->bhq", pq, z)[..., None] + 1e-6
        o = num / den
        return (lambda x, *d: x.transpose(*d))(o, 0, 2, 1, 3).reshape(B, S, D) @ wo

    def _B_ref(x, w_r, w_gate, w_up, w_down):
        B, S, D = x.shape
        C = 1
        r = x @ w_r
        idx = jnp.argsort(-r, axis=-1)[:, :C]
        idx_e = jnp.repeat(idx.reshape(B, C, 1), D, axis=2)
        x_sel = jnp.take_along_axis(x, idx_e, axis=1)
        g = _silu(x_sel @ w_gate)
        u = x_sel @ w_up
        y = (g * u) @ w_down
        r_sel = _sigmoid(jnp.take_along_axis(r, idx, axis=1))
        y = y * r_sel.reshape(B, C, 1)
        b_off = (jnp.arange(B) * S).reshape(B, 1)
        flat_idx = (idx + b_off).reshape(B * C)
        zero = (x * 0.0).reshape(B * S, D)
        upd = _scatter_add(zero, flat_idx, y.reshape(B * C, D), axis=0)
        return x + upd.reshape(B, S, D)

    x = A_x
    g = _sigmoid((x * gate_w).sum(-1, keepdims=True))
    a = _A_ref(x, A_wqkv, A_wo)
    b = _B_ref(x, B_w_r, B_w_gate, B_w_up, B_w_down)
    return g * a + (1 - g) * b
```

```python
import os
import jax
import jax.numpy as jnp
from jax import lax
import jax.experimental.pallas as pl
import jax.experimental.pallas.tpu as pltpu

S, D, F, H, DH = 2048, 1024, 3584, 32, 32
T = 512
NT = S // T
TP = 256
GM = int(os.environ.get('GM', 4))
RC = int(os.environ.get('RC', 32))
NC = 4
GC = D // NC
FC = F // NC
f32, bf16 = jnp.float32, jnp.bfloat16
NT_DIMS = (((1,), (1,)), ((), ()))
TN_DIMS = (((0,), (0,)), ((), ()))
AB = os.environ.get('AB', '')


def _phi(t):
    return jnp.where(t > 0, t + 1.0, jnp.exp(t)) + 1e-6


def _loop(name, lo, hi, body, carry):
    if name in os.environ.get('UN', ''):
        for i in range(lo, hi):
            carry = body(i, carry)
        return carry
    return lax.fori_loop(lo, hi, body, carry)


def _lanes(v, n):
    return jnp.concatenate([v] * n, axis=1)


def _matvec(w_ref, col_ref, r_lo, r_hi, cols, acc=None, rc=64, after=None):
    for r in range(r_lo, r_hi, rc):
        col = col_ref[pl.ds(r, rc), :]
        if after is not None:
            col = jnp.where(after[0], jnp.concatenate([after[1]] * (rc // 8), axis=0), col)
        if 'nomul' in AB:
            p = w_ref[pl.ds(r, rc), :].astype(f32)
            p = jnp.where(after[0][:, :1], _lanes(col, cols // 128), p) if 'sel' in AB else p
        else:
            p = w_ref[pl.ds(r, rc), :].astype(f32) * _lanes(col, cols // 128)
        p = jnp.sum(p.reshape(rc // 8, 8, cols), axis=0)
        acc = p if acc is None else acc + p
    return acc


def _kernel(ax_h, wqkv_h, wo_h, wr_ref, wg_h, wu_h, wd_h, gw_ref, out_h,
            x_v, w_v, wo_v, wg_v, wu_v, wd_v, wkT_v, wqT_v, pkT_v, G_v, m_v, z_v, g_v, pqn_v,
            xcol_v, hcol_v, gu_v, ob_v, sems, ksem, xsem, gsem, usem, dsem, osem):
    class _N:
        def start(self): pass
        def wait(self): pass
    def mk(src, dst, sem):
        return _N() if 'nodma' in AB else pltpu.make_async_copy(src, dst, sem)
    c_wq = mk(wqkv_h.at[:, pl.ds(0, D)], w_v.at[0], sems.at[0])
    c_wk = lambda c: mk(wqkv_h.at[:, pl.ds(D + c * GC, GC)], w_v.at[1, :, pl.ds(c * GC, GC)], ksem.at[c])
    c_wv = mk(wqkv_h.at[:, pl.ds(2 * D, D)], w_v.at[2], sems.at[2])
    c_wo = mk(wo_h, wo_v, sems.at[3])

    def rows(i, n):
        return pl.ds(pl.multiple_of(i * n, n), n)
    c_x = lambda i: mk(ax_h.at[0, rows(i, T)], x_v.at[rows(i, T)], xsem.at[i])
    c_wg = lambda j: mk(wg_h.at[:, rows(j, FC)], wg_v.at[j], gsem.at[j])
    c_wu = lambda j: mk(wu_h.at[:, rows(j, FC)], wu_v.at[j], usem.at[j])
    c_wd = lambda j: mk(wd_h.at[rows(j, FC)], wd_v.at[j], dsem.at[j])

    c_wk(0).start(); c_x(0).start(); c_wk(1).start()
    wr = wr_ref[...].astype(f32).reshape(1, D)
    gw = gw_ref[...].astype(f32).reshape(1, D)
    er = lax.broadcasted_iota(jnp.int32, (16, D), 0)
    wkT_v[pl.ds(0, 16), :] = jnp.where(er == 0, gw, jnp.where(er == 1, wr, 0.0)).astype(bf16)

    def gate_and_route(extra, t0, carry):
        best, bidx = carry
        g_v[pl.ds(t0, 128), :] = jnp.broadcast_to(jax.nn.sigmoid(extra[0:1]), (128, 128)).T
        r = extra[1:2].astype(bf16).astype(f32)
        upd = r > best
        ii = lax.broadcasted_iota(jnp.int32, (1, 128), 1) + t0
        return jnp.where(upd, r, best), jnp.where(upd, ii, bidx)

    carry = (jnp.full((1, 128), -jnp.inf, f32), lax.broadcasted_iota(jnp.int32, (1, 128), 1))
    c_wk(0).wait()
    c_wk(2).start(); c_wk(3).start()
    wkT_v[pl.ds(16, GC), :] = w_v[1, :, pl.ds(0, GC)].T
    c_x(0).wait()
    for c in range(NC):
        sl = pl.ds(c * GC, GC)
        if c + 1 < NC:
            c_wk(c + 1).wait()
            c_x(c + 1).start()
            wkT_v[pl.ds(16 + (c + 1) * GC, GC), :] = w_v[1, :, pl.ds((c + 1) * GC, GC)].T
        else:
            c_wq.start()
        lo = 0 if c == 0 else 16 + c * GC
        kT = lax.dot_general(wkT_v[pl.ds(lo, 16 + (c + 1) * GC - lo), :], x_v[pl.ds(0, T), :], NT_DIMS,
                             preferred_element_type=f32)
        if c == 0:
            for l in range(T // 128):
                carry = gate_and_route(kT[:16, l * 128:(l + 1) * 128], l * 128, carry)
            kT = kT[16:]
        pk = _phi(kT)
        pkT_v[sl, pl.ds(0, T)] = pk.astype(bf16)
        z_v[sl, :] = sum(pk[:, l * 128:(l + 1) * 128] for l in range(1, T // 128)) + pk[:, 0:128]

    def k_tile(i, carry):
        c_x(i).wait()
        c_wg(i - 1).start(); c_wu(i - 1).start()
        for l in range(T // 128):
            t0 = pl.multiple_of(i * T + l * 128, 128)
            kT = lax.dot_general(wkT_v[...], x_v[pl.ds(t0, 128), :], NT_DIMS, preferred_element_type=f32)
            carry = gate_and_route(kT[:16], t0, carry)
            pk = _phi(kT[16:])
            pkT_v[:, pl.ds(t0, 128)] = pk.astype(bf16)
            z_v[...] += pk
        return carry

    best, bidx = _loop('K', 1, 1 if 'noK' in AB else NT, k_tile, carry)
    c_wq.wait()
    c_wg(NC - 1).start(); c_wu(NC - 1).start(); c_wv.start(); c_wo.start()

    top = jnp.max(best, axis=1, keepdims=True)
    idx = jnp.min(jnp.where(best == top, bidx, S - 1), axis=1, keepdims=True)[0, 0]
    idx = jnp.clip(idx, 0, S - 1)
    base = pl.multiple_of((idx // 16) * 16, 16)
    grp = x_v[pl.ds(base, 16), :].astype(f32)
    sel = lax.broadcasted_iota(jnp.int32, (16, D), 0) == idx - base
    xsel = jnp.sum(jnp.where(sel, grp, 0.0), axis=0, keepdims=True)
    r_sel = jax.nn.sigmoid(jnp.sum(xsel * wr, axis=-1, keepdims=True).astype(bf16).astype(f32))
    xcol_v[...] = jnp.broadcast_to(xsel, (128, D)).T
    z_v[...] = jnp.broadcast_to(jnp.sum(z_v[...], axis=-1, keepdims=True), (D, 128))
    t_idx = idx // T
    tile_row = lambda s: pl.multiple_of(jnp.where(s == NT - 1, t_idx, jnp.where(s >= t_idx, s + 1, s)) * T, T)

    def q_post(qT, zb):
        n = qT.shape[0]
        pq = _phi(qT)
        den = jnp.sum((pq * zb).reshape(n // DH, DH, -1), axis=1, keepdims=True) + 1e-6
        return (pq.reshape(n // DH, DH, -1) * (1.0 / den)).reshape(n, -1).astype(bf16).T

    def q_chunk(s, l):
        t0 = pl.multiple_of(tile_row(s) + l * 128, 128)
        qT = lax.dot_general(wqT_v[...], x_v[pl.ds(t0, 128), :], NT_DIMS, preferred_element_type=f32)
        pqn_v[s % 2, pl.ds(l * 128, 128), :] = q_post(qT, z_v[...])

    for c in range(NC):
        sl = pl.ds(c * GC, GC)
        wqT_v[sl, :] = w_v[0, :, sl].T
    for l in range(T // 128):
        q_chunk(0, l)

    never = jnp.full((RC, 128), idx, jnp.int32) < 0

    def g_body(j, _):
        c_wg(j).wait(); c_wu(j).wait()
        c_wd(j).start()
        for which in range(2):
            cols = pl.ds(pl.multiple_of(j * GC + which * 128, 128), 128)
            Gc = jnp.dot(pkT_v[...], x_v[:, cols], preferred_element_type=f32)
            G_v[:, cols] = Gc.astype(bf16)
            for r in range(0, RC if 'noffn' in AB else (D // 2 if 'half' in AB else D), RC):
                gu_v[j, which, pl.ds(r // RC * 8, 8), :] = _matvec(
                    (wg_v, wu_v)[which].at[j], xcol_v, r, r + RC, FC, None, RC, after=(never, Gc[r:r + 8]))
        return 0

    _loop('G', 0, 0 if 'noG' in AB else NC, g_body, 0)

    def ffn_down(s, c, yacc, dep):
        for r in range(c * 128, (c + 1) * 128, RC):
            k = (r - c * 128) * dep.shape[0] // 128
            yacc = _matvec(wd_v.at[s], hcol_v.at[s], r, r + RC, D, yacc, RC, after=(never, dep[k:k + 8, :128]))
        return yacc

    def o_chunk(s, c, m0, m, y=None):
        sl = pl.ds(c * 128, 128)
        r0 = pl.multiple_of(tile_row(s) + m0, m)
        a = jnp.dot(pqn_v[s % 2, pl.ds(m0, m), :], m_v[:, sl], preferred_element_type=f32)
        b = x_v[pl.ds(r0, m), sl].astype(f32)
        if y is not None:
            hit = lax.broadcasted_iota(jnp.int32, (m, 128), 0) == idx - r0
            b = jnp.where(hit, b + y[:, c * 128:(c + 1) * 128], b)
        gt = g_v[pl.ds(r0, m), :]
        ob_v[s, pl.ds(m0, m), sl] = (gt * a + (1.0 - gt) * b).astype(bf16)
        return a

    def c_out(s, m0, m, k):
        return pltpu.make_async_copy(ob_v.at[s, pl.ds(m0, m)],
                                     out_h.at[0, pl.ds(pl.multiple_of(tile_row(s) + m0, m), m)], osem.at[k])

    c_wv.wait(); c_wo.wait(); c_wd(0).wait()
    for j in range(NC):
        gg = jnp.sum(gu_v[j, 0], axis=0, keepdims=True)
        uu = jnp.sum(gu_v[j, 1], axis=0, keepdims=True)
        hcol_v[j] = jnp.broadcast_to(gg * jax.nn.sigmoid(gg) * uu, (128, FC)).T
    ri = lax.broadcasted_iota(jnp.int32, (128, 128), 0) // DH
    ci = lax.broadcasted_iota(jnp.int32, (128, 128), 1) // DH
    yacc = jnp.zeros((8, D), f32)
    for g in range(D // 128):
        sg = pl.ds(g * 128, 128)
        kv = jnp.dot(G_v[sg, :], w_v[2, :, sg], preferred_element_type=f32)
        if g < FC // 128:
            yacc = ffn_down(0, g, yacc, kv)
        kv = jnp.where(ri == ci, kv, 0.0).astype(bf16)
        m_v[sg, :] = jnp.dot(kv, wo_v[sg, :], preferred_element_type=f32).astype(bf16)

    def q_body(s, yacc):
        c_wd(s).wait()
        for l in range(T // 128):
            q_chunk(s, l)
        for c in range(D // 128):
            a = o_chunk(s - 1, c, 0, T)
            if c < FC // 128:
                yacc = ffn_down(s, c, yacc, a)
        c_out(s - 1, 0, T, s - 1).start()
        return yacc

    yacc = _loop('Q', 1, 1 if 'noQ' in AB else NT, q_body, yacc)
    y = jnp.sum(yacc, axis=0, keepdims=True) * r_sel
    for p in range(T // TP):
        for c in range(D // 128):
            o_chunk(NT - 1, c, p * TP, TP, y)
        c_out(NT - 1, p * TP, TP, NT - 1 + p).start()
    if 'noQ' not in AB:
        for s in range(NT - 1):
            c_out(s, 0, T, s).wait()
    for p in range(T // TP):
        c_out(NT - 1, p * TP, TP, NT - 1 + p).wait()


@jax.jit
def pallas_gated_mix__linear_attn_block__moe_arch_mod__prompt_kernel(
        A_x, A_wqkv, A_wo, B_x, B_w_r, B_w_gate, B_w_up, B_w_down, gate_w):
    del B_x
    hbm = pl.BlockSpec(memory_space=pl.ANY)
    vm = pl.BlockSpec(memory_space=pltpu.VMEM)
    dma = pltpu.SemaphoreType.DMA
    return pl.pallas_call(
        _kernel,
        in_specs=[hbm, hbm, hbm, vm, hbm, hbm, hbm, vm],
        out_specs=hbm,
        out_shape=jax.ShapeDtypeStruct((1, S, D), bf16),
        scratch_shapes=[
            pltpu.VMEM((S, D), bf16), pltpu.VMEM((3, D, D), bf16), pltpu.VMEM((D, D), bf16),
            pltpu.VMEM((NC, D, FC), bf16), pltpu.VMEM((NC, D, FC), bf16), pltpu.VMEM((NC, FC, D), bf16),
            pltpu.VMEM((D + 16, D), bf16), pltpu.VMEM((D, D), bf16), pltpu.VMEM((D, S), bf16), pltpu.VMEM((D, D), bf16),
            pltpu.VMEM((D, D), bf16), pltpu.VMEM((D, 128), f32), pltpu.VMEM((S, 128), f32),
            pltpu.VMEM((2, T, D), bf16),
            pltpu.VMEM((D, 128), f32), pltpu.VMEM((NC, FC, 128), f32), pltpu.VMEM((NC, 2, D // RC * 8, FC), f32),
            pltpu.VMEM((NT, T, D), bf16),
            dma((4,)), dma((NC,)), dma((NT,)), dma((NC,)), dma((NC,)), dma((NC,)), dma((NT - 1 + T // TP,)),
        ],
        compiler_params=pltpu.CompilerParams(vmem_limit_bytes=100 * 1024 * 1024),
    )(A_x, A_wqkv, A_wo, B_w_r, B_w_gate, B_w_up, B_w_down, gate_w)
```

```python
import jax
import jax.numpy as jnp
from jax import lax
import jax.experimental.pallas as pl
import jax.experimental.pallas.tpu as pltpu

S, D, F, H, DH = 2048, 1024, 3584, 32, 32
T = 512
RC = 32
LAST = ((0,3,0,S),(3,6,0,S),(6,7,0,S),(7,8,0,1536),(7,8,1536,512))
YC = 3
KN = 128
NC = 4
GC = D // NC
FC = F // NC
f32, bf16 = jnp.float32, jnp.bfloat16
NT_DIMS = (((1,), (1,)), ((), ()))


def _phi(t):
    return jnp.exp(jnp.minimum(t, 0.0)) + (jnp.maximum(t, 0.0) + 1e-6)


def _lanes(v, n):
    return jnp.concatenate([v] * n, axis=1)


def _matvec(w_ref, col_ref, r_lo, r_hi, cols, acc=None, rc=64, after=None):
    for r in range(r_lo, r_hi, rc):
        col = col_ref[pl.ds(r, rc), :]
        if after is not None:
            col = jnp.where(after[0], jnp.concatenate([after[1]] * (rc // 8), axis=0), col)
        p = w_ref[pl.ds(r, rc), :].astype(f32) * _lanes(col, cols // 128)
        p = jnp.sum(p.reshape(rc // 8, 8, cols), axis=0)
        acc = p if acc is None else acc + p
    return acc


def _kernel(ax_h, wqkv_h, wo_h, wr_h, wg_h, wu_h, wd_h, gw_h, out_h,
            x_v, w_v, wo_v, wg_v, wu_v, wd_v, gw_v, wr_v, wkT_v, wqT_v, pkT_v, G_v, m_v, z_v, g_v, pqn_v,
            xcol_v, hcol_v, gu_v, ob_v, sems):
    n_sem = [0]

    def copy(src, dst):
        n_sem[0] += 1
        return pltpu.make_async_copy(src, dst, sems.at[n_sem[0] - 1])

    c_gw, c_wr = copy(gw_h, gw_v), copy(wr_h, wr_v)
    c_wk = [copy(wqkv_h.at[:, pl.ds(D + c * GC, GC)], w_v.at[1, :, pl.ds(c * GC, GC)]) for c in range(NC)]
    c_wq = copy(wqkv_h.at[:, pl.ds(0, D)], w_v.at[0])
    c_wv = copy(wqkv_h.at[:, pl.ds(2 * D, D)], w_v.at[2])
    c_wo, c_wg, c_wu, c_wd = copy(wo_h, wo_v), copy(wg_h, wg_v), copy(wu_h, wu_v), copy(wd_h, wd_v)
    x_cuts = (0, T // 2, T, 2 * T, 3 * T, S)
    c_x = [copy(ax_h.at[0, pl.ds(lo, hi - lo)], x_v.at[pl.ds(lo, hi - lo)])
           for lo, hi in zip(x_cuts[:-1], x_cuts[1:])]

    def gate_and_route(extra, t0, carry):
        best, bidx = carry
        g_v[pl.ds(t0, 128), :] = jnp.broadcast_to(jax.nn.sigmoid(extra[0:1]), (128, 128)).T
        r = extra[1:2].astype(bf16).astype(f32)
        upd = r > best
        ii = lax.broadcasted_iota(jnp.int32, (1, 128), 1) + t0
        return jnp.where(upd, r, best), jnp.where(upd, ii, bidx)

    def transpose_wk(c):
        wkT_v[pl.ds(16 + c * GC, GC), :] = w_v[1, :, pl.ds(c * GC, GC)].T

    def k_block(c_lo, c_hi, t0, n, carry):
        lo = 0 if c_lo == 0 else 16 + c_lo * GC
        kT = lax.dot_general(wkT_v[pl.ds(lo, 16 + c_hi * GC - lo), :], x_v[pl.ds(t0, n), :], NT_DIMS,
                             preferred_element_type=f32)
        if c_lo == 0:
            for l in range(0, n, 128):
                carry = gate_and_route(kT[:16, l:l + 128], t0 + l, carry)
            kT = kT[16:]
        pk = _phi(kT)
        sl = pl.ds(c_lo * GC, (c_hi - c_lo) * GC)
        pkT_v[sl, pl.ds(t0, n)] = pk.astype(bf16)
        zs = pk[:, 0:128]
        for l in range(128, n, 128):
            zs = zs + pk[:, l:l + 128]
        z_v[sl, :] = zs if t0 == 0 else z_v[sl, :] + zs
        return carry

    for c in (c_gw, c_wr, c_wk[0], c_wk[1], c_x[0], c_x[1], c_wk[2], c_wk[3], *c_x[2:],
              c_wq, c_wg, c_wu, c_wv, c_wo, c_wd):
        c.start()
    c_gw.wait(); c_wr.wait(); c_wk[0].wait()
    gw = gw_v[...].astype(f32).reshape(1, D)
    wr = wr_v[...].astype(f32).reshape(1, D)
    er = lax.broadcasted_iota(jnp.int32, (16, D), 0)
    wkT_v[pl.ds(0, 16), :] = jnp.where(er == 0, gw, jnp.where(er == 1, wr, 0.0)).astype(bf16)
    carry = (jnp.full((1, 128), -jnp.inf, f32), lax.broadcasted_iota(jnp.int32, (1, 128), 1))
    transpose_wk(0)
    c_wk[1].wait()
    transpose_wk(1)
    c_x[0].wait()
    carry = k_block(0, 2, 0, T // 2, carry)
    c_x[1].wait(); c_wk[2].wait()
    transpose_wk(2)
    carry = k_block(0, 2, T // 2, T // 2, carry)
    c_wk[3].wait()
    transpose_wk(3)
    carry = k_block(2, 3, 0, T, carry)
    carry = k_block(3, 4, 0, T, carry)
    c_x[2].wait()
    for t0 in range(T, S, KN):
        if t0 == 2 * T:
            c_x[3].wait(); c_x[4].wait()
        carry = k_block(0, NC, t0, KN, carry)
    best, bidx = carry
    c_wq.wait()
    c_wg.wait()

    top = jnp.max(best, axis=1, keepdims=True)
    idx = jnp.min(jnp.where(best == top, bidx, S - 1), axis=1, keepdims=True)[0, 0]
    idx = jnp.clip(idx, 0, S - 1)
    base = pl.multiple_of((idx // 16) * 16, 16)
    grp = x_v[pl.ds(base, 16), :].astype(f32)
    sel = lax.broadcasted_iota(jnp.int32, (16, D), 0) == idx - base
    xsel = jnp.sum(jnp.where(sel, grp, 0.0), axis=0, keepdims=True)
    r_sel = jax.nn.sigmoid(jnp.sum(xsel * wr, axis=-1, keepdims=True).astype(bf16).astype(f32))
    xcol_v[...] = jnp.broadcast_to(xsel, (128, D)).T
    z_v[...] = jnp.broadcast_to(jnp.sum(z_v[...], axis=-1, keepdims=True), (D, 128))

    def q_block(t0):
        qT = lax.dot_general(wqT_v[...], x_v[pl.ds(t0, 128), :], NT_DIMS, preferred_element_type=f32)
        pq = _phi(qT)
        den = jnp.sum((pq * z_v[...]).reshape(H, DH, 128), axis=1, keepdims=True) + 1e-6
        pqn = (pq.reshape(H, DH, 128) * (1.0 / den)).reshape(D, 128)
        pqn_v[pl.ds(t0, 128), :] = pqn.astype(bf16).T
        return qT

    for c in range(NC):
        sl = pl.ds(c * GC, GC)
        wqT_v[sl, :] = w_v[0, :, sl].T
    for t0 in range(0, T, 128):
        q_block(t0)

    never = jnp.full((RC, 128), idx, jnp.int32) < 0
    for j in range(D // 128):
        if j == NC:
            c_wu.wait()
        cols = pl.ds(j * 128, 128)
        Gc = jnp.dot(pkT_v[...], x_v[:, cols], preferred_element_type=f32)
        G_v[:, cols] = Gc.astype(bf16)
        w_ref = (wg_v, wu_v)[j // NC].at[:, pl.ds(j % NC * FC, FC)]
        for r in range(0, D, RC):
            gu_v[j, pl.ds(r // RC * 8, 8), :] = _matvec(w_ref, xcol_v, r, r + RC, FC, None, RC,
                                                        after=(never, Gc[r:r + 8]))
    c_wv.wait(); c_wo.wait()

    for j in range(NC):
        gg = jnp.sum(gu_v[j], axis=0, keepdims=True)
        uu = jnp.sum(gu_v[NC + j], axis=0, keepdims=True)
        hcol_v[pl.ds(j * FC, FC), :] = jnp.broadcast_to(gg * jax.nn.sigmoid(gg) * uu, (128, FC)).T
    ri = lax.broadcasted_iota(jnp.int32, (128, 128), 0) // DH
    ci = lax.broadcasted_iota(jnp.int32, (128, 128), 1) // DH
    for g in range(D // 128):
        sg = pl.ds(g * 128, 128)
        kv = jnp.dot(G_v[sg, :], w_v[2, :, sg], preferred_element_type=f32)
        kv = jnp.where(ri == ci, kv, 0.0).astype(bf16)
        m_v[sg, :] = jnp.dot(kv, wo_v[sg, :], preferred_element_type=f32).astype(bf16)

    def ffn_down(c_lo, c_hi, k, n, yacc, dep):
        lo, hi = F // RC * k // n, F // RC * (k + 1) // n
        w_ref = wd_v.at[:, pl.ds(c_lo * 128, (c_hi - c_lo) * 128)]
        for p in range(lo, hi):
            r = (p - lo) * (dep.shape[0] // 8 // (hi - lo)) * 8
            yacc = _matvec(w_ref, hcol_v, p * RC, (p + 1) * RC, (c_hi - c_lo) * 128, yacc, RC,
                           after=(never, dep[r:r + 8]))
        return yacc

    def route_update(c_lo, c_hi, yacc):
        sl = pl.ds(c_lo * 128, (c_hi - c_lo) * 128)
        y = jnp.sum(yacc, axis=0, keepdims=True) * r_sel
        grp = x_v[pl.ds(base, 16), sl].astype(f32)
        hit = lax.broadcasted_iota(jnp.int32, grp.shape, 0) == idx - base
        x_v[pl.ds(base, 16), sl] = jnp.where(hit, grp + y, grp).astype(bf16)

    c_wd.wait()
    yacc = None
    n_blk = (S - T) // 128
    for k in range(n_blk):
        yacc = ffn_down(0, YC, k, n_blk, yacc, q_block(T + k * 128))
    route_update(0, YC, yacc)

    c_o = []
    yacc = None
    for k, (lo, hi, r0, nr) in enumerate(LAST):
        rs = pl.ds(r0, nr)
        for c in range(lo, hi):
            sl = pl.ds(c * 128, 128)
            a = jnp.dot(pqn_v[rs, :], m_v[:, sl], preferred_element_type=f32)
            gt = g_v[rs, :]
            ob_v[rs, sl] = (gt * a + (1.0 - gt) * x_v[rs, sl].astype(f32)).astype(bf16)
            if c < YC:
                yacc = ffn_down(YC, D // 128, c, YC, yacc, a)
            if c == YC - 1:
                route_update(YC, D // 128, yacc)
        sl = pl.ds(lo * 128, (hi - lo) * 128)
        c_o.append(pltpu.make_async_copy(ob_v.at[rs, sl], out_h.at[0, rs, sl], sems.at[n_sem[0] + k]))
        c_o[-1].start()
    for c in c_o:
        c.wait()


@jax.jit
def pallas_gated_mix__linear_attn_block__moe_arch_mod__prompt_kernel(
        A_x, A_wqkv, A_wo, B_x, B_w_r, B_w_gate, B_w_up, B_w_down, gate_w):
    del B_x
    hbm = pl.BlockSpec(memory_space=pl.ANY)
    return pl.pallas_call(
        _kernel,
        in_specs=[hbm] * 8,
        out_specs=hbm,
        out_shape=jax.ShapeDtypeStruct((1, S, D), bf16),
        scratch_shapes=[
            pltpu.VMEM((S, D), bf16), pltpu.VMEM((3, D, D), bf16), pltpu.VMEM((D, D), bf16),
            pltpu.VMEM((D, F), bf16), pltpu.VMEM((D, F), bf16), pltpu.VMEM((F, D), bf16),
            pltpu.VMEM((D,), bf16), pltpu.VMEM((D,), bf16),
            pltpu.VMEM((D + 16, D), bf16), pltpu.VMEM((D, D), bf16), pltpu.VMEM((D, S), bf16),
            pltpu.VMEM((D, D), bf16), pltpu.VMEM((D, D), bf16), pltpu.VMEM((D, 128), f32),
            pltpu.VMEM((S, 128), f32), pltpu.VMEM((S, D), bf16),
            pltpu.VMEM((D, 128), f32), pltpu.VMEM((F, 128), f32),
            pltpu.VMEM((2 * NC, D // RC * 8, FC), f32), pltpu.VMEM((S, D), bf16),
            pltpu.SemaphoreType.DMA((32,)),
        ],
        compiler_params=pltpu.CompilerParams(vmem_limit_bytes=100 * 1024 * 1024),
    )(A_x, A_wqkv, A_wo, B_w_r, B_w_gate, B_w_up, B_w_down, gate_w)
```

```python
import jax
import jax.numpy as jnp
from jax import lax
import jax.experimental.pallas as pl
import jax.experimental.pallas.tpu as pltpu

S, D, F, H, DH = 2048, 1024, 3584, 32, 32
T = 512
RC = 32
LAST = ((0,3,0,S),(3,6,0,S),(6,7,0,S),(7,8,0,1536),(7,8,1536,512))
YC = 3
KN = 128
NC = 4
GC = D // NC
FC = F // NC
f32, bf16 = jnp.float32, jnp.bfloat16
NT_DIMS = (((1,), (1,)), ((), ()))


def _phi(t):
    return jnp.exp(jnp.minimum(t, 0.0)) + (jnp.maximum(t, 0.0) + 1e-6)


def _lanes(v, n):
    return jnp.concatenate([v] * n, axis=1)


def _matvec(w_ref, col_ref, r_lo, r_hi, cols, acc=None, rc=64, after=None):
    for r in range(r_lo, r_hi, rc):
        col = col_ref[pl.ds(r, rc), :]
        if after is not None:
            col = jnp.where(after[0], jnp.concatenate([after[1]] * (rc // 8), axis=0), col)
        p = w_ref[pl.ds(r, rc), :].astype(f32) * _lanes(col, cols // 128)
        p = jnp.sum(p.reshape(rc // 8, 8, cols), axis=0)
        acc = p if acc is None else acc + p
    return acc


def _kernel(ax_h, wqkv_h, wo_h, wr_h, wg_h, wu_h, wd_h, gw_h, out_h,
            x_v, w_v, wo_v, wg_v, wu_v, wd_v, gw_v, wr_v, wkT_v, wqT_v, pkT_v, G_v, m_v, z_v, g_v, pqn_v,
            xcol_v, hcol_v, gu_v, ob_v, sems):
    n_sem = [0]

    def copy(src, dst):
        n_sem[0] += 1
        return pltpu.make_async_copy(src, dst, sems.at[n_sem[0] - 1])

    c_gw, c_wr = copy(gw_h, gw_v), copy(wr_h, wr_v)
    c_wk = [copy(wqkv_h.at[:, pl.ds(D + c * GC, GC)], w_v.at[1, :, pl.ds(c * GC, GC)]) for c in range(NC)]
    c_wq = copy(wqkv_h.at[:, pl.ds(0, D)], w_v.at[0])
    c_wv = copy(wqkv_h.at[:, pl.ds(2 * D, D)], w_v.at[2])
    c_wo, c_wg, c_wu, c_wd = copy(wo_h, wo_v), copy(wg_h, wg_v), copy(wu_h, wu_v), copy(wd_h, wd_v)
    x_cuts = (0, T // 2, T, 2 * T, 3 * T, S)
    c_x = [copy(ax_h.at[0, pl.ds(lo, hi - lo)], x_v.at[pl.ds(lo, hi - lo)])
           for lo, hi in zip(x_cuts[:-1], x_cuts[1:])]

    def gate_and_route(extra, t0, carry):
        best, bidx = carry
        g_v[pl.ds(t0, 128), :] = jnp.broadcast_to(jax.nn.sigmoid(extra[0:1]), (128, 128)).T
        r = extra[1:2].astype(bf16).astype(f32)
        upd = r > best
        ii = lax.broadcasted_iota(jnp.int32, (1, 128), 1) + t0
        return jnp.where(upd, r, best), jnp.where(upd, ii, bidx)

    def transpose_wk(c):
        wkT_v[pl.ds(16 + c * GC, GC), :] = w_v[1, :, pl.ds(c * GC, GC)].T

    def k_block(c_lo, c_hi, t0, n, carry):
        lo = 0 if c_lo == 0 else 16 + c_lo * GC
        kT = lax.dot_general(wkT_v[pl.ds(lo, 16 + c_hi * GC - lo), :], x_v[pl.ds(t0, n), :], NT_DIMS,
                             preferred_element_type=f32)
        if c_lo == 0:
            for l in range(0, n, 128):
                carry = gate_and_route(kT[:16, l:l + 128], t0 + l, carry)
            kT = kT[16:]
        pk = _phi(kT)
        sl = pl.ds(c_lo * GC, (c_hi - c_lo) * GC)
        pkT_v[sl, pl.ds(t0, n)] = pk.astype(bf16)
        zs = pk[:, 0:128]
        for l in range(128, n, 128):
            zs = zs + pk[:, l:l + 128]
        z_v[sl, :] = zs if t0 == 0 else z_v[sl, :] + zs
        return carry

    for c in (c_gw, c_wr, c_wk[0], c_x[0], c_wk[1], c_x[1], c_wk[2], c_wk[3], *c_x[2:],
              c_wq, c_wg, c_wu, c_wv, c_wo, c_wd):
        c.start()
    c_gw.wait(); c_wr.wait(); c_wk[0].wait()
    gw = gw_v[...].astype(f32).reshape(1, D)
    wr = wr_v[...].astype(f32).reshape(1, D)
    er = lax.broadcasted_iota(jnp.int32, (16, D), 0)
    wkT_v[pl.ds(0, 16), :] = jnp.where(er == 0, gw, jnp.where(er == 1, wr, 0.0)).astype(bf16)
    carry = (jnp.full((1, 128), -jnp.inf, f32), lax.broadcasted_iota(jnp.int32, (1, 128), 1))
    transpose_wk(0)
    c_x[0].wait()
    carry = k_block(0, 1, 0, T // 2, carry)
    c_wk[1].wait()
    transpose_wk(1)
    carry = k_block(1, 2, 0, T // 2, carry)
    c_x[1].wait()
    carry = k_block(0, 1, T // 2, T // 2, carry)
    c_wk[2].wait()
    transpose_wk(2)
    carry = k_block(1, 2, T // 2, T // 2, carry)
    c_wk[3].wait()
    transpose_wk(3)
    carry = k_block(2, 3, 0, T, carry)
    carry = k_block(3, 4, 0, T, carry)
    c_x[2].wait()
    for t0 in range(T, S, KN):
        if t0 == 2 * T:
            c_x[3].wait(); c_x[4].wait(); c_wq.wait()
        if t0 >= 3 * T:
            sl = pl.ds((t0 - 3 * T) // 128 * GC, GC)
            wqT_v[sl, :] = w_v[0, :, sl].T
        carry = k_block(0, NC, t0, KN, carry)
    best, bidx = carry
    c_wg.wait()

    top = jnp.max(best, axis=1, keepdims=True)
    idx = jnp.min(jnp.where(best == top, bidx, S - 1), axis=1, keepdims=True)[0, 0]
    idx = jnp.clip(idx, 0, S - 1)
    base = pl.multiple_of((idx // 16) * 16, 16)
    grp = x_v[pl.ds(base, 16), :].astype(f32)
    sel = lax.broadcasted_iota(jnp.int32, (16, D), 0) == idx - base
    xsel = jnp.sum(jnp.where(sel, grp, 0.0), axis=0, keepdims=True)
    r_sel = jax.nn.sigmoid(jnp.sum(xsel * wr, axis=-1, keepdims=True).astype(bf16).astype(f32))
    xcol_v[...] = jnp.broadcast_to(xsel, (128, D)).T
    z_v[...] = jnp.broadcast_to(jnp.sum(z_v[...], axis=-1, keepdims=True), (D, 128))

    def q_block(t0):
        qT = lax.dot_general(wqT_v[...], x_v[pl.ds(t0, 128), :], NT_DIMS, preferred_element_type=f32)
        pq = _phi(qT)
        den = jnp.sum((pq * z_v[...]).reshape(H, DH, 128), axis=1, keepdims=True) + 1e-6
        pqn = (pq.reshape(H, DH, 128) * (1.0 / den)).reshape(D, 128)
        pqn_v[pl.ds(t0, 128), :] = pqn.astype(bf16).T
        return qT

    for t0 in range(0, T, 128):
        q_block(t0)

    never = jnp.full((RC, 128), idx, jnp.int32) < 0
    for j in range(D // 128):
        if j == NC:
            c_wu.wait()
        cols = pl.ds(j * 128, 128)
        Gc = jnp.dot(pkT_v[...], x_v[:, cols], preferred_element_type=f32)
        G_v[:, cols] = Gc.astype(bf16)
        w_ref = (wg_v, wu_v)[j // NC].at[:, pl.ds(j % NC * FC, FC)]
        for r in range(0, D, RC):
            gu_v[j, pl.ds(r // RC * 8, 8), :] = _matvec(w_ref, xcol_v, r, r + RC, FC, None, RC,
                                                        after=(never, Gc[r:r + 8]))
    c_wv.wait(); c_wo.wait()

    for j in range(NC):
        gg = jnp.sum(gu_v[j], axis=0, keepdims=True)
        uu = jnp.sum(gu_v[NC + j], axis=0, keepdims=True)
        hcol_v[pl.ds(j * FC, FC), :] = jnp.broadcast_to(gg * jax.nn.sigmoid(gg) * uu, (128, FC)).T
    ri = lax.broadcasted_iota(jnp.int32, (128, 128), 0) // DH
    ci = lax.broadcasted_iota(jnp.int32, (128, 128), 1) // DH
    for g in range(D // 128):
        sg = pl.ds(g * 128, 128)
        kv = jnp.dot(G_v[sg, :], w_v[2, :, sg], preferred_element_type=f32)
        kv = jnp.where(ri == ci, kv, 0.0).astype(bf16)
        m_v[sg, :] = jnp.dot(kv, wo_v[sg, :], preferred_element_type=f32).astype(bf16)

    def ffn_down(c_lo, c_hi, k, n, yacc, dep):
        lo, hi = F // RC * k // n, F // RC * (k + 1) // n
        w_ref = wd_v.at[:, pl.ds(c_lo * 128, (c_hi - c_lo) * 128)]
        for p in range(lo, hi):
            r = (p - lo) * (dep.shape[0] // 8 // (hi - lo)) * 8
            yacc = _matvec(w_ref, hcol_v, p * RC, (p + 1) * RC, (c_hi - c_lo) * 128, yacc, RC,
                           after=(never, dep[r:r + 8]))
        return yacc

    def route_update(c_lo, c_hi, yacc):
        sl = pl.ds(c_lo * 128, (c_hi - c_lo) * 128)
        y = jnp.sum(yacc, axis=0, keepdims=True) * r_sel
        grp = x_v[pl.ds(base, 16), sl].astype(f32)
        hit = lax.broadcasted_iota(jnp.int32, grp.shape, 0) == idx - base
        x_v[pl.ds(base, 16), sl] = jnp.where(hit, grp + y, grp).astype(bf16)

    c_wd.wait()
    yacc = None
    n_blk = (S - T) // 128
    for k in range(n_blk):
        yacc = ffn_down(0, YC, k, n_blk, yacc, q_block(T + k * 128))
    route_update(0, YC, yacc)

    c_o = []
    yacc = None
    for k, (lo, hi, r0, nr) in enumerate(LAST):
        rs = pl.ds(r0, nr)
        for c in range(lo, hi):
            sl = pl.ds(c * 128, 128)
            a = jnp.dot(pqn_v[rs, :], m_v[:, sl], preferred_element_type=f32)
            gt = g_v[rs, :]
            ob_v[rs, sl] = (gt * a + (1.0 - gt) * x_v[rs, sl].astype(f32)).astype(bf16)
            if c < YC:
                yacc = ffn_down(YC, D // 128, c, YC, yacc, a)
            if c == YC - 1:
                route_update(YC, D // 128, yacc)
        sl = pl.ds(lo * 128, (hi - lo) * 128)
        c_o.append(pltpu.make_async_copy(ob_v.at[rs, sl], out_h.at[0, rs, sl], sems.at[n_sem[0] + k]))
        c_o[-1].start()
    for c in c_o:
        c.wait()


@jax.jit
def pallas_gated_mix__linear_attn_block__moe_arch_mod__prompt_kernel(
        A_x, A_wqkv, A_wo, B_x, B_w_r, B_w_gate, B_w_up, B_w_down, gate_w):
    del B_x
    hbm = pl.BlockSpec(memory_space=pl.ANY)
    return pl.pallas_call(
        _kernel,
        in_specs=[hbm] * 8,
        out_specs=hbm,
        out_shape=jax.ShapeDtypeStruct((1, S, D), bf16),
        scratch_shapes=[
            pltpu.VMEM((S, D), bf16), pltpu.VMEM((3, D, D), bf16), pltpu.VMEM((D, D), bf16),
            pltpu.VMEM((D, F), bf16), pltpu.VMEM((D, F), bf16), pltpu.VMEM((F, D), bf16),
            pltpu.VMEM((D,), bf16), pltpu.VMEM((D,), bf16),
            pltpu.VMEM((D + 16, D), bf16), pltpu.VMEM((D, D), bf16), pltpu.VMEM((D, S), bf16),
            pltpu.VMEM((D, D), bf16), pltpu.VMEM((D, D), bf16), pltpu.VMEM((D, 128), f32),
            pltpu.VMEM((S, 128), f32), pltpu.VMEM((S, D), bf16),
            pltpu.VMEM((D, 128), f32), pltpu.VMEM((F, 128), f32),
            pltpu.VMEM((2 * NC, D // RC * 8, FC), f32), pltpu.VMEM((S, D), bf16),
            pltpu.SemaphoreType.DMA((32,)),
        ],
        compiler_params=pltpu.CompilerParams(vmem_limit_bytes=100 * 1024 * 1024),
    )(A_x, A_wqkv, A_wo, B_w_r, B_w_gate, B_w_up, B_w_down, gate_w)
```

```python
import jax
import jax.numpy as jnp
from jax import lax
import jax.experimental.pallas as pl
import jax.experimental.pallas.tpu as pltpu

S, D, F, H, DH = 2048, 1024, 3584, 32, 32
L = 128
T = 512
KT = (S - T) // 2
NC = 4
GC = D // NC
FC = F // NC
RC = 32
YW = 3 * L
PIECES = ((0, 3, 0, S), (3, 6, 0, S), (6, 7, 0, S), (7, 8, 0, 1536), (7, 8, 1536, 512))
f32, bf16 = jnp.float32, jnp.bfloat16
NT_DIMS = (((1,), (1,)), ((), ()))


def _phi(t):
    return jnp.exp(jnp.minimum(t, 0.0)) + (jnp.maximum(t, 0.0) + 1e-6)


def _matvec_slice(w_ref, col_ref, r, never, after):
    cols = w_ref.shape[1]
    col = jnp.where(never, jnp.concatenate([after] * (RC // 8), axis=0), col_ref[pl.ds(r, RC), :])
    p = w_ref[pl.ds(r, RC), :].astype(f32) * jnp.concatenate([col] * (cols // L), axis=1)
    return jnp.sum(p.reshape(RC // 8, 8, cols), axis=0)


def _kernel(ax_h, wqkv_h, wo_h, wr_h, wg_h, wu_h, wd_h, gw_h, out_h,
            x_v, w_v, wo_v, wgu_v, wd_v, gw_v, wr_v, wkT_v, wqT_v, pkT_v, G_v, m_v, z_v, g_v, pqn_v,
            xcol_v, hcol_v, gu_v, ob_v, sems):
    n_sem = [0]

    def copy(src, dst):
        n_sem[0] += 1
        return pltpu.make_async_copy(src, dst, sems.at[n_sem[0] - 1])

    c_gw, c_wr = copy(gw_h, gw_v), copy(wr_h, wr_v)
    c_wk = [copy(wqkv_h.at[:, pl.ds(D + c * GC, GC)], w_v.at[1, :, pl.ds(c * GC, GC)]) for c in range(NC)]
    c_wq = copy(wqkv_h.at[:, pl.ds(0, D)], w_v.at[0])
    c_wv = copy(wqkv_h.at[:, pl.ds(2 * D, D)], w_v.at[2])
    c_wo, c_wg, c_wu, c_wd = copy(wo_h, wo_v), copy(wg_h, wgu_v.at[0]), copy(wu_h, wgu_v.at[1]), copy(wd_h, wd_v)
    x_cuts = (0, T // 2, T, T + KT, S)
    c_x = [copy(ax_h.at[0, pl.ds(lo, hi - lo)], x_v.at[pl.ds(lo, hi - lo)])
           for lo, hi in zip(x_cuts[:-1], x_cuts[1:])]
    for c in (c_gw, c_wr, c_wk[0], c_x[0], c_wk[1], c_x[1], c_wk[2], c_wk[3], c_x[2], c_x[3],
              c_wq, c_wg, c_wu, c_wv, c_wo, c_wd):
        c.start()

    def gate_and_route(extra, t0, carry):
        best, bidx = carry
        g_v[pl.ds(t0, L), :] = jnp.broadcast_to(jax.nn.sigmoid(extra[0:1]), (L, L)).T
        r = extra[1:2].astype(bf16).astype(f32)
        upd = r > best
        ii = lax.broadcasted_iota(jnp.int32, (1, L), 1) + t0
        return jnp.where(upd, r, best), jnp.where(upd, ii, bidx)

    def transpose_wk(c):
        wkT_v[pl.ds(16 + c * GC, GC), :] = w_v[1, :, pl.ds(c * GC, GC)].T

    def k_block(c_lo, c_hi, t0, n, carry, first=False):
        lo = 0 if c_lo == 0 else 16 + c_lo * GC
        kT = lax.dot_general(wkT_v[pl.ds(lo, 16 + c_hi * GC - lo), :], x_v[pl.ds(t0, n), :], NT_DIMS,
                             preferred_element_type=f32)
        if c_lo == 0:
            for l in range(0, n, L):
                carry = gate_and_route(kT[:16, l:l + L], t0 + l, carry)
            kT = kT[16:]
        pk = _phi(kT)
        sl = pl.ds(c_lo * GC, (c_hi - c_lo) * GC)
        pkT_v[sl, pl.ds(t0, n)] = pk.astype(bf16)
        zs = pk[:, 0:L]
        for l in range(L, n, L):
            zs = zs + pk[:, l:l + L]
        z_v[sl, :] = zs if first else z_v[sl, :] + zs
        return carry

    c_gw.wait(); c_wr.wait(); c_wk[0].wait()
    gw = gw_v[...].astype(f32).reshape(1, D)
    wr = wr_v[...].astype(f32).reshape(1, D)
    er = lax.broadcasted_iota(jnp.int32, (16, D), 0)
    wkT_v[pl.ds(0, 16), :] = jnp.where(er == 0, gw, jnp.where(er == 1, wr, 0.0)).astype(bf16)
    carry = (jnp.full((1, L), -jnp.inf, f32), lax.broadcasted_iota(jnp.int32, (1, L), 1))
    transpose_wk(0)
    c_x[0].wait()
    carry = k_block(0, 1, 0, T // 2, carry, first=True)
    c_wk[1].wait()
    transpose_wk(1)
    carry = k_block(1, 2, 0, T // 2, carry, first=True)
    c_x[1].wait()
    carry = k_block(0, 1, T // 2, T // 2, carry)
    c_wk[2].wait()
    transpose_wk(2)
    carry = k_block(1, 2, T // 2, T // 2, carry)
    c_wk[3].wait()
    transpose_wk(3)
    carry = k_block(2, 3, 0, T, carry, first=True)
    carry = k_block(3, 4, 0, T, carry, first=True)

    def k_half(i, carry):
        pl.when(i == 0)(c_x[2].wait)
        pl.when(i == 1)(c_x[3].wait)
        pl.when(i == 1)(c_wq.wait)
        for l in range(0, KT, L):
            if l // L < NC:
                sl = pl.ds(l // L * GC, GC)
                wqT_v[sl, :] = w_v[1 - i, :, sl].T
            carry = k_block(0, NC, pl.multiple_of(T + i * KT + l, L), L, carry)
        return carry

    best, bidx = lax.fori_loop(0, 2, k_half, carry)

    top = jnp.max(best, axis=1, keepdims=True)
    idx = jnp.min(jnp.where(best == top, bidx, S - 1), axis=1, keepdims=True)[0, 0]
    idx = jnp.clip(idx, 0, S - 1)
    base = pl.multiple_of((idx // 16) * 16, 16)
    grp = x_v[pl.ds(base, 16), :].astype(f32)
    sel = lax.broadcasted_iota(jnp.int32, (16, D), 0) == idx - base
    xsel = jnp.sum(jnp.where(sel, grp, 0.0), axis=0, keepdims=True)
    r_sel = jax.nn.sigmoid(jnp.sum(xsel * wr, axis=-1, keepdims=True).astype(bf16).astype(f32))
    xcol_v[...] = jnp.broadcast_to(xsel, (L, D)).T
    z_v[...] = jnp.broadcast_to(jnp.sum(z_v[...], axis=-1, keepdims=True), (D, L))

    def q_block(t0):
        qT = lax.dot_general(wqT_v[...], x_v[pl.ds(t0, L), :], NT_DIMS, preferred_element_type=f32)
        pq = _phi(qT)
        den = jnp.sum((pq * z_v[...]).reshape(H, DH, L), axis=1, keepdims=True) + 1e-6
        pqn = (pq.reshape(H, DH, L) * (1.0 / den)).reshape(D, L)
        pqn_v[pl.ds(t0, L), :] = pqn.astype(bf16).T
        return qT

    for t0 in range(0, T, L):
        q_block(t0)
    c_wg.wait()

    never = jnp.full((RC, L), idx, jnp.int32) < 0
    for j in range(D // L):
        if j == NC:
            c_wu.wait()
        cols = pl.ds(j * L, L)
        Gc = jnp.dot(pkT_v[...], x_v[:, cols], preferred_element_type=f32)
        G_v[:, cols] = Gc.astype(bf16)
        w_ref = wgu_v.at[j // NC, :, pl.ds(j % NC * FC, FC)]
        for r in range(0, D, RC):
            gu_v[j, pl.ds(r // RC * 8, 8), :] = _matvec_slice(w_ref, xcol_v, r, never, Gc[r:r + 8])
    c_wv.wait(); c_wo.wait()

    for j in range(NC):
        gg = jnp.sum(gu_v[j], axis=0, keepdims=True)
        uu = jnp.sum(gu_v[NC + j], axis=0, keepdims=True)
        hcol_v[pl.ds(j * FC, FC), :] = jnp.broadcast_to(gg * jax.nn.sigmoid(gg) * uu, (L, FC)).T
    ri = lax.broadcasted_iota(jnp.int32, (L, L), 0) // DH
    ci = lax.broadcasted_iota(jnp.int32, (L, L), 1) // DH
    for g in range(D // L):
        sg = pl.ds(g * L, L)
        kv = jnp.dot(G_v[sg, :], w_v[2, :, sg], preferred_element_type=f32)
        kv = jnp.where(ri == ci, kv, 0.0).astype(bf16)
        m_v[sg, :] = jnp.dot(kv, wo_v[sg, :], preferred_element_type=f32).astype(bf16)

    def ffn_down(cols, k, n, yacc, dep):
        lo, hi = F // RC * k // n, F // RC * (k + 1) // n
        for p in range(lo, hi):
            r = (p - lo) * (dep.shape[0] // 8 // (hi - lo)) * 8
            part = _matvec_slice(wd_v.at[:, cols], hcol_v, p * RC, never, dep[r:r + 8])
            yacc = part if yacc is None else yacc + part
        return yacc

    def route_update(cols, yacc):
        y = jnp.sum(yacc, axis=0, keepdims=True) * r_sel
        rows = x_v[pl.ds(base, 16), cols].astype(f32)
        hit = lax.broadcasted_iota(jnp.int32, rows.shape, 0) == idx - base
        x_v[pl.ds(base, 16), cols] = jnp.where(hit, rows + y, rows).astype(bf16)

    c_wd.wait()
    yacc = None
    n_blk = (S - T) // L
    for k in range(n_blk):
        yacc = ffn_down(pl.ds(0, YW), k, n_blk, yacc, q_block(T + k * L))
    route_update(pl.ds(0, YW), yacc)

    c_o = []
    yacc = None
    rest = pl.ds(YW, D - YW)
    for lo, hi, r0, nr in PIECES:
        rs = pl.ds(r0, nr)
        for c in range(lo, hi):
            sl = pl.ds(c * L, L)
            a = jnp.dot(pqn_v[rs, :], m_v[:, sl], preferred_element_type=f32)
            gt = g_v[rs, :]
            ob_v[rs, sl] = (gt * a + (1.0 - gt) * x_v[rs, sl].astype(f32)).astype(bf16)
            if c < YW // L:
                yacc = ffn_down(rest, c, YW // L, yacc, a)
            if c == YW // L - 1:
                route_update(rest, yacc)
        sl = pl.ds(lo * L, (hi - lo) * L)
        c_o.append(copy(ob_v.at[rs, sl], out_h.at[0, rs, sl]))
        c_o[-1].start()
    for c in c_o:
        c.wait()


@jax.jit
def pallas_gated_mix__linear_attn_block__moe_arch_mod__prompt_kernel(
        A_x, A_wqkv, A_wo, B_x, B_w_r, B_w_gate, B_w_up, B_w_down, gate_w):
    del B_x
    hbm = pl.BlockSpec(memory_space=pl.ANY)
    return pl.pallas_call(
        _kernel,
        in_specs=[hbm] * 8,
        out_specs=hbm,
        out_shape=jax.ShapeDtypeStruct((1, S, D), bf16),
        scratch_shapes=[
            pltpu.VMEM((S, D), bf16),
            pltpu.VMEM((3, D, D), bf16),
            pltpu.VMEM((D, D), bf16),
            pltpu.VMEM((2, D, F), bf16),
            pltpu.VMEM((F, D), bf16),
            pltpu.VMEM((D,), bf16), pltpu.VMEM((D,), bf16),
            pltpu.VMEM((D + 16, D), bf16),
            pltpu.VMEM((D, D), bf16),
            pltpu.VMEM((D, S), bf16),
            pltpu.VMEM((D, D), bf16),
            pltpu.VMEM((D, D), bf16),
            pltpu.VMEM((D, L), f32),
            pltpu.VMEM((S, L), f32),
            pltpu.VMEM((S, D), bf16),
            pltpu.VMEM((D, L), f32),
            pltpu.VMEM((F, L), f32),
            pltpu.VMEM((2 * NC, D // RC * 8, FC), f32),
            pltpu.VMEM((S, D), bf16),
            pltpu.SemaphoreType.DMA((16 + len(PIECES),)),
        ],
        compiler_params=pltpu.CompilerParams(vmem_limit_bytes=100 * 1024 * 1024),
    )(A_x, A_wqkv, A_wo, B_w_r, B_w_gate, B_w_up, B_w_down, gate_w)
```
